```python
import os as _os
_os.environ.setdefault('JAX_PLATFORMS', 'cpu')
import jax
import jax.numpy as jnp

def _softmax(x, axis=-1):
    return jax.nn.softmax(x, axis=axis)

def _gelu(x):
    return jax.nn.gelu(x, approximate=True)

def _silu(x):
    return jax.nn.silu(x)

def _sigmoid(x):
    return jax.nn.sigmoid(x)

def _layernorm(x, axis=-1, eps=1e-05):
    m = jnp.mean(x, axis=axis, keepdims=True)
    v = jnp.var(x, axis=axis, keepdims=True)
    return (x - m) / jnp.sqrt(v + eps)

def _scatter_add(tgt, idx, src, axis=0):
    return tgt.at[idx].add(src)

def _segment_sum(src, seg, n):
    return jax.ops.segment_sum(src, seg, n)

class _Rng:

    def __init__(self, key):
        self._k = key

    def _next(self):
        self._k, sub = jax.random.split(self._k)
        return sub

    def normal(self, shape):
        return jax.random.normal(self._next(), shape, dtype=jnp.bfloat16)

    def randint(self, lo, hi, shape):
        return jax.random.randint(self._next(), shape, lo, hi, dtype=jnp.int32)

    def uniform(self, shape, lo=0.0, hi=1.0):
        return jax.random.uniform(self._next(), shape, jnp.bfloat16, lo, hi)

    def permutation(self, n):
        return jax.random.permutation(self._next(), n)
kernel_name = 'gated_mix__memory_aug_recurrent_mem_tr__glu_gated_geglu__prompt'

def setup_inputs():
    _rng = _Rng(jax.random.key(int.from_bytes(__import__("os").urandom(4), "little")))
    _w = lambda a: (lambda t: t.astype(jnp.bfloat16) if jnp.issubdtype(t.dtype, jnp.floating) else t)(jnp.asarray(a))

    def _A_setup():
        B, S, Dm = (1, 2048, 640)
        H, Dh = (32, 128)
        M, seg = (8, 32)
        seg = min(seg, S)
        S = S // seg * seg
        return {'x': _w((lambda *s: _rng.normal(s) * 0.05)(B, S, Dm)), 'mem0': _w((lambda *s: _rng.normal(s) * 0.4)(B, M, Dm)), 'Wq': _w((lambda *s: _rng.normal(s) * 3.2)(Dm, H, Dh) * Dm ** (-0.5)), 'Wk': _w((lambda *s: _rng.normal(s) * 3.2)(Dm, H, Dh) * Dm ** (-0.5)), 'Wv': _w((lambda *s: _rng.normal(s) * 0.4)(Dm, H, Dh) * Dm ** (-0.5)), 'Wo': _w((lambda *s: _rng.normal(s) * 0.4)(H, Dh, Dm) * (H * Dh) ** (-0.5)), 'seg_len': seg}
    _A_in = _A_setup()

    def _B_setup():
        B, S, Dm, Df = (1, 2048, 640, 1728)
        return {'x': _w((lambda *s: _rng.normal(s) * 0.05)(B, S, Dm)), 'w_gate': _w((lambda *s: _rng.normal(s) * 1.6)(Dm, Df) * Dm ** (-0.5)), 'w_up': _w((lambda *s: _rng.normal(s) * 1.6)(Dm, Df) * Dm ** (-0.5)), 'w_down': _w((lambda *s: _rng.normal(s) * 1.6)(Df, Dm) * Df ** (-0.5))}
    _B_in = _B_setup()
    return {'A_x': _A_in['x'], 'A_mem0': _A_in['mem0'], 'A_Wq': _A_in['Wq'], 'A_Wk': _A_in['Wk'], 'A_Wv': _A_in['Wv'], 'A_Wo': _A_in['Wo'], 'A_seg_len': _A_in['seg_len'], 'B_x': _B_in['x'], 'B_w_gate': _B_in['w_gate'], 'B_w_up': _B_in['w_up'], 'B_w_down': _B_in['w_down'], 'gate_w': _w((lambda *s: _rng.normal(s) * 0.05)(640) * 16.0)}

def reference(A_x, A_mem0, A_Wq, A_Wk, A_Wv, A_Wo, A_seg_len, B_x, B_w_gate, B_w_up, B_w_down, gate_w):

    def _A_ref(x, mem0, Wq, Wk, Wv, Wo, seg_len):
        B, S, Dm = x.shape
        H, Dh = (Wq.shape[1], Wq.shape[2])
        M = mem0.shape[1]
        scale = Dh ** (-0.5)
        n_seg = S // seg_len
        L = M + seg_len
        idx = jnp.arange(L)
        mask = (idx[:, None] < M) | (idx[:, None] >= idx[None, :])
        mem = mem0
        outs = []
        for s in range(n_seg):
            xs = x[:, s * seg_len:(s + 1) * seg_len, :].copy()
            h = jnp.concatenate([mem, xs], axis=1)
            q = jnp.einsum('btd,dhe->bhte', h, Wq)
            k = jnp.einsum('btd,dhe->bhte', h, Wk)
            v = jnp.einsum('btd,dhe->bhte', h, Wv)
            scores = jnp.einsum('bhqe,bhke->bhqk', q, k) * scale
            scores = jnp.where(mask[None, None], scores, -1000000000.0)
            p = _softmax(scores, axis=-1)
            o = jnp.einsum('bhqk,bhke->bhqe', p, v)
            o = jnp.einsum('bhte,hed->btd', o, Wo)
            mem = o[:, :M, :].copy()
            outs.append(o[:, M:, :])
        return jnp.concatenate(outs, axis=1)

    def _B_ref(x, w_gate, w_up, w_down):
        g = jnp.einsum('bsd,df->bsf', x, w_gate)
        u = jnp.einsum('bsd,df->bsf', x, w_up)
        h = _gelu(g) * u
        return jnp.einsum('bsf,fd->bsd', h, w_down)
    x = A_x
    g = _sigmoid((x * gate_w).sum(-1, keepdims=True))
    a = _A_ref(x, A_mem0, A_Wq, A_Wk, A_Wv, A_Wo, A_seg_len)
    b = _B_ref(x, B_w_gate, B_w_up, B_w_down)
    return g * a + (1 - g) * b
```

```python
import functools
import jax
import jax.numpy as jnp
from jax import lax
import jax.experimental.pallas as pl
import jax.experimental.pallas.tpu as pltpu

F32 = jnp.float32
BF16 = jnp.bfloat16
U32 = jnp.uint32


def _gelu_tanh(x):
    c = 0.7978845608028654
    return 0.5 * x * (1.0 + jnp.tanh(c * (x + 0.044715 * (x * x * x))))


def _recip(d):
    r = pl.reciprocal(d, approx=True)
    return r * (2.0 - d * r)


def _bf(w32):
    return pltpu.bitcast(w32, BF16)


def _impl(A_x, A_mem0, A_Wq, A_Wk, A_Wv, A_Wo, A_seg_len, B_x, B_w_gate, B_w_up, B_w_down, gate_w,
              DS=1, DPV=3, NREL=2, FC=256, GB0=512, NITRUN=32, WSTART=1, WPTS=(0, 1, 3)):
    B, S, Dm = A_x.shape
    H, Dh = A_Wq.shape[1], A_Wq.shape[2]
    M = A_mem0.shape[1]
    SEG = 32
    L = M + SEG
    NSEG = S // SEG
    Df = B_w_gate.shape[1]
    scale = Dh ** (-0.5)
    NP = H // 2
    PW = 6 * Dh
    GB = 256
    NGB = S // GB
    NIT = NSEG // 2
    D2 = Dm // 2

    def kernel(x_hbm, mem0_hbm, wq_hbm, wk_hbm, wv_hbm, wo_hbm, wgT_hbm, wuT_hbm, wd_hbm, gw_hbm,
               out_hbm,
               x_ref, mem0_ref, wst, wg32, wu32, wd32, gw_ref, out_v,
               wqkv32, wo32, bacc, qkv_sv, o_sv, sems, osem):
        fchunks = [(f0, min(FC, Df - f0)) for f0 in range(0, Df, FC)]
        NFC = len(fchunks)
        cp = lambda src, dst, i: pltpu.make_async_copy(src, dst, sems.at[i])
        c_x0 = cp(x_hbm.at[pl.ds(0, GB0)], x_ref.at[pl.ds(0, GB0)], 0)
        c_xr = cp(x_hbm.at[pl.ds(GB0, S - GB0)], x_ref.at[pl.ds(GB0, S - GB0)], 1)
        c_gw = cp(gw_hbm, gw_ref, 2)
        c_m0 = cp(mem0_hbm, mem0_ref, 3)
        c_wo = cp(wo_hbm.bitcast(U32), wo32, 4)
        c_w = []
        for t, w_hbm in enumerate((wq_hbm, wk_hbm, wv_hbm)):
            w32 = w_hbm.bitcast(U32)
            c_w += [cp(w32.at[:, r, :], wst.at[t, r], 5 + t) for r in range(2 * NP)]
        c_w.append(c_wo)
        c_f = []
        for t, (w_hbm, w_v) in enumerate(((wgT_hbm, wg32), (wuT_hbm, wu32), (wd_hbm, wd32))):
            w32 = w_hbm.bitcast(U32)
            c_f.append([cp(w32.at[pl.ds(f0 // 2, fw // 2)], w_v.at[pl.ds(f0 // 2, fw // 2)], 8 + t * NFC + c)
                        for c, (f0, fw) in enumerate(fchunks)])

        NT = (((1,), (1,)), ((), ()))

        def relay(t, j):
            off = pl.multiple_of(j * PW + t * 2 * Dh, 2 * Dh)
            for i0 in range(0, D2, 64):
                a = wst[t, j, i0:i0 + 64, :]
                b = wst[t, NP + j, i0:i0 + 64, :]
                lo = (a & U32(0xFFFF)) | (b << 16)
                hi = (a >> 16) | (b & U32(0xFFFF0000))
                wqkv32[i0:i0 + 64, pl.ds(off, Dh)] = lo
                wqkv32[i0:i0 + 64, pl.ds(off + Dh, Dh)] = hi

        def geglu(r0, nrows, customize, jobs):
            xb = x_ref[pl.ds(r0, nrows), :]
            nslots = 3 * NFC
            slot = [0]
            def filler():
                lo = slot[0] * len(jobs) // nslots
                hi = (slot[0] + 1) * len(jobs) // nslots
                for j in jobs[lo:hi]:
                    j()
                slot[0] += 1
            hs = {}
            b = None
            for c in range(NFC + 1):
                if c < NFC:
                    f0, fw = fchunks[c]
                    customize(0, c)
                    g = lax.dot_general(xb, _bf(wg32[f0 // 2:(f0 + fw) // 2, :]), NT, preferred_element_type=F32)
                    filler()
                    customize(1, c)
                    u = lax.dot_general(xb, _bf(wu32[f0 // 2:(f0 + fw) // 2, :]), NT, preferred_element_type=F32)
                    filler()
                    hs[c] = (_gelu_tanh(g) * u).astype(BF16)
                if c >= 1:
                    f0, fw = fchunks[c - 1]
                    customize(2, c - 1)
                    r = jnp.dot(hs.pop(c - 1), _bf(wd32[f0 // 2:(f0 + fw) // 2, :]), preferred_element_type=F32)
                    b = r if b is None else b + r
                    filler()
            gw = gw_ref[...].astype(F32)
            gate = jax.nn.sigmoid(jnp.sum(xb.astype(F32) * gw, axis=-1, keepdims=True))
            bacc[pl.ds(r0, nrows), :] = (1.0 - gate) * b

        c_x0.start()
        c_f[0][0].start(); c_f[1][0].start()
        c_gw.start(); c_m0.start()
        for c in range(1, NFC):
            c_f[0][c].start(); c_f[1][c].start(); c_f[2][c - 1].start()
        c_f[2][NFC - 1].start()
        c_xr.start()
        if WSTART == 0:
            for c in c_w: c.start()
        c_x0.wait(); c_gw.wait(); c_m0.wait()
        def cust0(kind, c):
            if kind == 0 and c in WPTS:
                nxt = [w for w in WPTS if w > c]
                end = nxt[0] if nxt else NFC + 1
                for cc in range(c, end):
                    if cc < NFC:
                        c_f[0][cc].wait(); c_f[1][cc].wait()
                    if cc >= 1:
                        c_f[2][cc - 1].wait()
                k = WPTS.index(c)
                if k >= 1 and k <= 2:
                    for cc in c_w[(k - 1) * 32:k * 32]:
                        cc.start()
        geglu(0, GB0, cust0, [])
        c_xr.wait()
        for cc in c_w[64:]:
            cc.start()
        gw = gw_ref[...].astype(F32)

        def geglu_loop(i, rel):
            r0 = pl.multiple_of(i * GB, GB)
            jobs = []
            if rel:
                k = i - (NGB - NREL)
                for t in range(3):
                    for c in range(NP // NREL):
                        jobs.append(functools.partial(relay, t, k * (NP // NREL) + c))
            geglu(r0, GB, lambda kind, c: None, jobs)

        lax.fori_loop(GB0 // GB, NGB - NREL, lambda i, c: (geglu_loop(i, False), c)[1], 0)
        for c in c_w: c.wait()
        lax.fori_loop(NGB - NREL, NGB, lambda i, c: (geglu_loop(i, True), c)[1], 0)

        ri = lax.broadcasted_iota(jnp.int32, (2 * L, 2 * L), 0)
        ci = lax.broadcasted_iota(jnp.int32, (2 * L, 2 * L), 1)
        rh = ri >= L
        ch = ci >= L
        rl = jnp.where(rh, ri - L, ri)
        cl = jnp.where(ch, ci - L, ci)
        mask = (rh == ch) & ((rl < M) | (rl >= cl))

        def seg_step(h, first):
            qkv_s, e_s, o2_s = {}, {}, {}
            acc = [None]

            def do_qkv(p):
                r = jnp.dot(h, _bf(wqkv32[:, p * PW:(p + 1) * PW]), preferred_element_type=F32)
                if first:
                    qkv_sv[:, p * PW:(p + 1) * PW] = r[L:L + 8]
                    qkv = r[0:L]
                else:
                    qkv = jnp.concatenate([r[0:M], qkv_sv[:, p * PW:(p + 1) * PW], r[M:]], axis=0)
                q = jnp.concatenate([qkv[:, 0:Dh], qkv[:, Dh:2 * Dh]], axis=0).astype(BF16)
                k = jnp.concatenate([qkv[:, 2 * Dh:3 * Dh], qkv[:, 3 * Dh:4 * Dh]], axis=0).astype(BF16)
                v = jnp.concatenate([qkv[:, 4 * Dh:5 * Dh], qkv[:, 5 * Dh:6 * Dh]], axis=0).astype(BF16)
                qkv_s[p] = (q, k, v)

            def do_s(p):
                q, k, v = qkv_s[p]
                sc = lax.dot_general(q, k, NT, preferred_element_type=F32) * scale
                sc = jnp.where(mask, sc, -1e9)
                mx = jnp.max(sc, axis=-1, keepdims=True)
                e = jnp.exp(sc - mx)
                den = jnp.sum(e, axis=-1, keepdims=True)
                e_s[p] = (e.astype(BF16), _recip(den))

            def do_pv(p):
                e, r = e_s.pop(p)
                v = qkv_s.pop(p)[2]
                o = jnp.dot(e, v, preferred_element_type=F32) * r
                o2 = jnp.concatenate([o[0:L], o[L:2 * L]], axis=1)
                if first:
                    o_sv[:, p * 2 * Dh:(p + 1) * 2 * Dh] = o2[L - 8:L]
                    o2_s[p] = o2[0:L - 8].astype(BF16)
                else:
                    o2_s[p] = jnp.concatenate([o2, o_sv[:, p * 2 * Dh:(p + 1) * 2 * Dh]], axis=0).astype(BF16)

            def do_wo(p):
                o2 = o2_s.pop(p)
                r = jnp.dot(o2, _bf(wo32[p * Dh:(p + 1) * Dh, :]), preferred_element_type=F32)
                acc[0] = r if acc[0] is None else acc[0] + r

            wo_next = 0
            for p in range(NP):
                do_qkv(p)
                if p - DS >= 0: do_s(p - DS)
                if p - DPV >= 0: do_pv(p - DPV)
            tail = []
            for t in range(NP, NP + DPV):
                if t - DS < NP: tail.append(('s', t - DS))
                tail.append(('pv', t - DPV))
            nwo = NP - DPV - wo_next
            per = max(1, nwo // len(tail))
            for kind, p in tail:
                for _ in range(per):
                    if wo_next < NP - DPV:
                        do_wo(wo_next); wo_next += 1
                (do_s if kind == 's' else do_pv)(p)
            while wo_next < NP:
                do_wo(wo_next); wo_next += 1
            return acc[0]

        def out_copy(i):
            r0 = pl.multiple_of(i * 2 * SEG, 2 * SEG)
            return pltpu.make_async_copy(out_v.at[pl.ds(r0, 2 * SEG)], out_hbm.at[pl.ds(r0, 2 * SEG)], osem)

        def pair_step(i, mem):
            r0 = pl.multiple_of(i * 2 * SEG, 2 * SEG)
            xf = x_ref[pl.ds(r0, 2 * SEG), :].astype(F32)
            hA = jnp.concatenate([mem, xf[0:SEG + 8]], axis=0).astype(BF16)
            aA = seg_step(hA, True)
            memB = aA[:M]
            hB = jnp.concatenate([memB, xf[SEG + 8:]], axis=0).astype(BF16)
            aB = seg_step(hB, False)
            a = jnp.concatenate([aA[M:], aB[L:L + 8], aB[M:L]], axis=0)
            gl = jnp.sum(xf * gw, axis=-1, keepdims=True)
            gate = jax.nn.sigmoid(gl)
            out_v[pl.ds(r0, 2 * SEG), :] = (gate * a + bacc[pl.ds(r0, 2 * SEG), :]).astype(out_v.dtype)
            out_copy(i).start()
            return aB[:M]

        lax.fori_loop(0, NITRUN, pair_step, mem0_ref[...].astype(F32))
        def wait_out(i, c):
            out_copy(i).wait()
            return c
        lax.fori_loop(0, NITRUN, wait_out, 0)

    any_spec = pl.BlockSpec(memory_space=pl.ANY)
    out = pl.pallas_call(
        kernel,
        out_shape=jax.ShapeDtypeStruct((S, Dm), BF16),
        in_specs=[any_spec] * 10,
        out_specs=any_spec,
        scratch_shapes=[
            pltpu.VMEM((S, Dm), BF16), pltpu.VMEM((M, Dm), BF16), pltpu.VMEM((3, H, D2, Dh), U32),
            pltpu.VMEM((Df // 2, Dm), U32), pltpu.VMEM((Df // 2, Dm), U32),
            pltpu.VMEM((Df // 2, Dm), U32), pltpu.VMEM((1, Dm), BF16), pltpu.VMEM((S, Dm), BF16),
            pltpu.VMEM((D2, 3 * H * Dh), U32), pltpu.VMEM((H * Dh // 2, Dm), U32),
            pltpu.VMEM((S, Dm), F32), pltpu.VMEM((8, 3 * H * Dh), F32), pltpu.VMEM((8, H * Dh), F32),
            pltpu.SemaphoreType.DMA((8 + 3 * (-(-Df // FC)),)), pltpu.SemaphoreType.DMA,
        ],
        compiler_params=pltpu.CompilerParams(vmem_limit_bytes=110 * 1024 * 1024),
    )(A_x.reshape(S, Dm), A_mem0.reshape(M, Dm), A_Wq.reshape(D2, 2 * H, Dh), A_Wk.reshape(D2, 2 * H, Dh),
      A_Wv.reshape(D2, 2 * H, Dh), A_Wo.reshape(H * Dh, Dm),
      B_w_gate.T, B_w_up.T, B_w_down, gate_w.reshape(1, Dm))
    return out.reshape(B, S, Dm)


@jax.jit
def pallas_gated_mix__memory_aug_recurrent_mem_tr__glu_gated_geglu__prompt_kernel(
    A_x: jax.Array,
    A_mem0: jax.Array,
    A_Wq: jax.Array,
    A_Wk: jax.Array,
    A_Wv: jax.Array,
    A_Wo: jax.Array,
    A_seg_len: jax.Array,
    B_x: jax.Array,
    B_w_gate: jax.Array,
    B_w_up: jax.Array,
    B_w_down: jax.Array,
    gate_w: jax.Array,
):
    return _impl(A_x, A_mem0, A_Wq, A_Wk, A_Wv, A_Wo, A_seg_len, B_x, B_w_gate, B_w_up, B_w_down, gate_w)
```

```python
import functools
import jax
import jax.numpy as jnp
from jax import lax
import jax.experimental.pallas as pl
import jax.experimental.pallas.tpu as pltpu

F32 = jnp.float32
BF16 = jnp.bfloat16
U32 = jnp.uint32


def _gelu_tanh(x):
    c = 0.7978845608028654
    return 0.5 * x * (1.0 + jnp.tanh(c * (x + 0.044715 * (x * x * x))))


def _recip(d):
    r = pl.reciprocal(d, approx=True)
    return r * (2.0 - d * r)


def _bf(w32):
    return pltpu.bitcast(w32, BF16)


def _impl(A_x, A_mem0, A_Wq, A_Wk, A_Wv, A_Wo, A_seg_len, B_x, B_w_gate, B_w_up, B_w_down, gate_w,
              DS=1, DPV=2, UNR=2, FC=256, GB0=512, NITRUN=32, WPTS=(0, 1, 2, 5, 9), WST=(1, 5), TAILA=(2, 3, 4), TAILB=(2, 2, 2),
              NTW=3, KSPLIT=1, QSPLIT=4, NOBC=True, GPRE=True):
    B, S, Dm = A_x.shape
    H, Dh = A_Wq.shape[1], A_Wq.shape[2]
    M = A_mem0.shape[1]
    SEG = 32
    L = M + SEG
    NSEG = S // SEG
    Df = B_w_gate.shape[1]
    scale = Dh ** (-0.5)
    NP = H // 2
    PW = 6 * Dh
    GB = 256
    NGB = S // GB
    NIT = NSEG // 2
    D2 = Dm // 2
    NG = NGB - GB0 // GB
    JG = 3 * NP // NG
    GPW = NP // JG
    fchunks = [(f0, min(FC, Df - f0)) for f0 in range(0, Df, FC)]
    NFC = len(fchunks)
    SEM_G = 5
    SEM_F = SEM_G + NG
    NSEM = SEM_F + 3 * NFC + 1

    def kernel(x_hbm, mem0_hbm, wq_hbm, wk_hbm, wv_hbm, wo_hbm, wgT_hbm, wuT_hbm, wd_hbm, gw_hbm,
               out_hbm,
               x32, mem0_ref, wst, wgu32, wd32, gw1_ref, gw_ref, out_v,
               wqkv32, wo32, bacc, gsv, qkv_sv, o_sv, sems, osem):
        cp = lambda src, dst, i: pltpu.make_async_copy(src, dst, sems.at[i])
        x32h = x_hbm.bitcast(U32)
        c_x0 = cp(x32h.at[pl.ds(0, GB0 // 4)], x32.at[pl.ds(0, GB0 // 4)], 0)
        c_x1 = cp(x32h.at[pl.ds(GB0 // 4, GB0 // 4)], x32.at[pl.ds(GB0 // 4, GB0 // 4)], NSEM - 1)
        c_xr = cp(x32h.at[pl.ds(GB0 // 2, (S - GB0) // 2)], x32.at[pl.ds(GB0 // 2, (S - GB0) // 2)], 1)
        def xrows(r0, n):
            if isinstance(r0, int):
                return _bf(x32[r0 // 2:(r0 + n) // 2, :])
            return _bf(x32[pl.ds(pl.multiple_of(r0 // 2, 8), n // 2), :])
        c_gw = cp(gw_hbm, gw1_ref, 2)
        c_m0 = cp(mem0_hbm, mem0_ref, 3)
        c_wo = cp(wo_hbm.bitcast(U32), wo32, 4)
        c_w = []
        for t, w_hbm in enumerate((wq_hbm, wk_hbm, wv_hbm)):
            w32 = w_hbm.bitcast(U32)
            for hf in range(GPW):
                gi = t * GPW + hf
                c_w.append([cp(w32.at[:, par * NP + hf * JG + jj, :], wst.at[gi, par * JG + jj], SEM_G + gi)
                            for jj in range(JG) for par in range(2)])
        wg32h, wu32h, wd32h = wgT_hbm.bitcast(U32), wuT_hbm.bitcast(U32), wd_hbm.bitcast(U32)
        c_f = [[], [], []]
        for c, (f0, fw) in enumerate(fchunks):
            c_f[0].append(cp(wg32h.at[pl.ds(f0 // 2, fw // 2)], wgu32.at[pl.ds(f0, fw // 2)], SEM_F + c))
            c_f[1].append(cp(wu32h.at[pl.ds(f0 // 2, fw // 2)], wgu32.at[pl.ds(f0 + fw // 2, fw // 2)], SEM_F + NFC + c))
            c_f[2].append(cp(wd32h.at[pl.ds(f0 // 2, fw // 2)], wd32.at[pl.ds(f0 // 2, fw // 2)], SEM_F + 2 * NFC + c))

        NT = (((1,), (1,)), ((), ()))

        def relay(gi, jj):
            t = gi // GPW
            hf = gi % GPW
            off = pl.multiple_of((hf * JG + jj) * PW + t * 2 * Dh, 2 * Dh)
            for i0 in range(0, D2, 64):
                a = wst[gi, jj, i0:i0 + 64, :]
                b = wst[gi, JG + jj, i0:i0 + 64, :]
                lo = (a & U32(0xFFFF)) | (b << 16)
                hi = (a >> 16) | (b & U32(0xFFFF0000))
                wqkv32[i0:i0 + 64, pl.ds(off, Dh)] = lo
                wqkv32[i0:i0 + 64, pl.ds(off + Dh, Dh)] = hi

        def geglu(r0, nrows, customize, jobs, ramp=False):
            nslots = 2 * NFC
            slot = [0]
            def filler():
                lo = slot[0] * len(jobs) // nslots
                hi = (slot[0] + 1) * len(jobs) // nslots
                for j in jobs[lo:hi]:
                    j()
                slot[0] += 1
            hs = {}
            b = None
            for c in range(NFC + 1):
                if c < NFC:
                    f0, fw = fchunks[c]
                    customize(('gu', c))
                    if ramp and c == 0:
                        hr = nrows // 2
                        gu0 = lax.dot_general(xrows(r0, hr), _bf(wgu32[f0:f0 + fw, :]), NT, preferred_element_type=F32)
                        c_x1.wait()
                        gu1 = lax.dot_general(xrows(r0 + hr, hr), _bf(wgu32[f0:f0 + fw, :]), NT, preferred_element_type=F32)
                        gu = jnp.concatenate([gu0, gu1], axis=0)
                    else:
                        gu = lax.dot_general(xrows(r0, nrows), _bf(wgu32[f0:f0 + fw, :]), NT, preferred_element_type=F32)
                    filler()
                    hs[c] = (_gelu_tanh(gu[:, :fw]) * gu[:, fw:]).astype(BF16)
                if c >= 1:
                    f0, fw = fchunks[c - 1]
                    hh = hs.pop(c - 1)
                    customize(('d', c - 1))
                    if c == NFC and fw % 128 != 0 and QSPLIT > 1:
                        k0 = fw // 128 * 128
                        r = jnp.dot(hh[:, :k0], _bf(wd32[f0 // 2:(f0 + k0) // 2, :]), preferred_element_type=F32)
                        b = b + r
                        wl = _bf(wd32[(f0 + k0) // 2:(f0 + fw) // 2, :])
                        qr = nrows // QSPLIT
                        r = jnp.concatenate([jnp.dot(hh[q * qr:(q + 1) * qr, k0:], wl, preferred_element_type=F32)
                                             for q in range(QSPLIT)], axis=0)
                    else:
                        r = jnp.dot(hh, _bf(wd32[f0 // 2:(f0 + fw) // 2, :]), preferred_element_type=F32)
                    b = r if b is None else b + r
                    filler()
            gate = jax.nn.sigmoid(jnp.sum(xrows(r0, nrows).astype(F32) * gw_ref[...], axis=-1, keepdims=True))
            bacc[pl.ds(r0, nrows), :] = (1.0 - gate) * b
            if GPRE:
                gsv[pl.ds(r0, nrows), :] = jnp.broadcast_to(gate, (nrows, 128))

        c_x0.start()
        c_f[0][0].start(); c_f[1][0].start()
        c_x1.start()
        c_gw.start(); c_m0.start()
        for c in range(1, NFC):
            c_f[0][c].start(); c_f[1][c].start(); c_f[2][c - 1].start()
        c_f[2][NFC - 1].start()
        c_xr.start()
        c_x0.wait()
        seq = [('gu', 0)]
        for c in range(1, NFC):
            seq += [('gu', c), ('d', c - 1)]
        seq.append(('d', NFC - 1))
        def cust0(item):
            n = seq.index(item)
            if n in WPTS:
                nxt = [w for w in WPTS if w > n]
                end = nxt[0] if nxt else len(seq)
                for kind, cc in seq[n:end]:
                    if kind == 'gu':
                        c_f[0][cc].wait(); c_f[1][cc].wait()
                    else:
                        c_f[2][cc].wait()
            if n == WPTS[1]:
                c_gw.wait(); c_m0.wait()
                gw_ref[...] = gw1_ref[...].astype(F32).reshape(1, Dm)
            if n in WST:
                k = WST.index(n)
                for gi in range(k * 2, k * 2 + 2):
                    for cc in c_w[gi]:
                        cc.start()
        geglu(0, GB0, cust0, [], ramp=True)
        c_xr.wait()
        for gi in range(4, NG):
            for cc in c_w[gi]:
                cc.start()
        c_wo.start()

        def geglu_loop(gi, carry):
            r0 = pl.multiple_of(GB0 + gi * GB, GB)
            pltpu.make_async_copy(wst.at[gi], wst.at[gi], sems.at[SEM_G + gi]).wait()
            jobs = [functools.partial(relay, gi, jj) for jj in range(JG)]
            geglu(r0, GB, lambda c: None, jobs)
            return carry

        lax.fori_loop(0, NG, geglu_loop, 0)
        c_wo.wait()

        ri = lax.broadcasted_iota(jnp.int32, (2 * L, 2 * L), 0)
        ci = lax.broadcasted_iota(jnp.int32, (2 * L, 2 * L), 1)
        rh = ri >= L
        ch = ci >= L
        rl = jnp.where(rh, ri - L, ri)
        cl = jnp.where(ch, ci - L, ci)
        mask = (rh == ch) & ((rl < M) | (rl >= cl))
        fill = jnp.where(rh == ch, -1e9, -jnp.inf).astype(F32)

        def seg_step(h, first, ksplit):
            qkv_s, e_s, o2_s = {}, {}, {}
            acc = [None]

            def do_qkv(p):
                if ksplit and p < KSPLIT:
                    r = None
                    for kk in range(Dm // 128):
                        rr = jnp.dot(h[:, kk * 128:(kk + 1) * 128],
                                     _bf(wqkv32[kk * 64:(kk + 1) * 64, p * PW:(p + 1) * PW]), preferred_element_type=F32)
                        r = rr if r is None else r + rr
                else:
                    r = jnp.dot(h, _bf(wqkv32[:, p * PW:(p + 1) * PW]), preferred_element_type=F32)
                if first:
                    qkv_sv[:, p * PW:(p + 1) * PW] = r[L:L + 8]
                    qkv = r[0:L]
                else:
                    qkv = jnp.concatenate([r[0:M], qkv_sv[:, p * PW:(p + 1) * PW], r[M:]], axis=0)
                q = jnp.concatenate([qkv[:, 0:Dh], qkv[:, Dh:2 * Dh]], axis=0).astype(BF16)
                k = jnp.concatenate([qkv[:, 2 * Dh:3 * Dh], qkv[:, 3 * Dh:4 * Dh]], axis=0).astype(BF16)
                v = jnp.concatenate([qkv[:, 4 * Dh:5 * Dh], qkv[:, 5 * Dh:6 * Dh]], axis=0).astype(BF16)
                qkv_s[p] = (q, k, v)

            def do_s(p):
                q, k, v = qkv_s[p]
                sc = lax.dot_general(q, k, NT, preferred_element_type=F32) * scale
                sc = jnp.where(mask, sc, fill)
                mx = jnp.max(sc, axis=-1, keepdims=True)
                e = jnp.exp(sc - mx)
                den = jnp.sum(e, axis=-1, keepdims=True)
                e_s[p] = (e.astype(BF16), _recip(den))

            def do_pv(p):
                e, r = e_s.pop(p)
                v = qkv_s.pop(p)[2]
                o = jnp.dot(e, v, preferred_element_type=F32) * r
                o2 = jnp.concatenate([o[0:L], o[L:2 * L]], axis=1)
                if first:
                    o_sv[:, p * 2 * Dh:(p + 1) * 2 * Dh] = o2[L - 8:L]
                    o2_s[p] = o2[0:L - 8].astype(BF16)
                else:
                    o2_s[p] = jnp.concatenate([o2, o_sv[:, p * 2 * Dh:(p + 1) * 2 * Dh]], axis=0).astype(BF16)

            def do_wo(p):
                o2 = o2_s.pop(p)
                r = jnp.dot(o2, _bf(wo32[p * Dh:(p + 1) * Dh, :]), preferred_element_type=F32)
                acc[0] = r if acc[0] is None else acc[0] + r

            wo_next = 0
            for p in range(NP):
                do_qkv(p)
                if p - DS >= 0: do_s(p - DS)
                if p - DPV >= 0: do_pv(p - DPV)
            tail = []
            for t in range(NP, NP + DPV):
                if t - DS < NP: tail.append(('s', t - DS))
                tail.append(('pv', t - DPV))
            for (kind, p), cnt in zip(tail, TAILA if first else TAILB):
                for _ in range(cnt):
                    do_wo(wo_next); wo_next += 1
                (do_s if kind == 's' else do_pv)(p)
            while wo_next < NP - NTW:
                do_wo(wo_next); wo_next += 1
            o2 = jnp.concatenate([o2_s.pop(p) for p in range(NP - NTW, NP)], axis=1)
            r = jnp.dot(o2, _bf(wo32[(NP - NTW) * Dh:NP * Dh, :]), preferred_element_type=F32)
            return acc[0] + r

        def out_copy(i):
            r0 = pl.multiple_of(i * 2 * SEG, 2 * SEG)
            return pltpu.make_async_copy(out_v.at[pl.ds(r0, 2 * SEG)], out_hbm.at[pl.ds(r0, 2 * SEG)], osem)

        def pair_step(i, mem, ksplit_a=False):
            r0 = pl.multiple_of(i * 2 * SEG, 2 * SEG)
            xf = xrows(r0, 2 * SEG).astype(F32)
            hA = jnp.concatenate([mem, xf[0:SEG + 8]], axis=0).astype(BF16)
            aA = seg_step(hA, True, ksplit_a)
            memB = aA[:M]
            hB = jnp.concatenate([memB, xf[SEG + 8:]], axis=0).astype(BF16)
            aB = seg_step(hB, False, True)
            a = jnp.concatenate([aA[M:], aB[L:L + 8], aB[M:L]], axis=0)
            if GPRE:
                g128 = gsv[pl.ds(r0, 2 * SEG), :]
                gate = jnp.concatenate([g128] * (Dm // 128), axis=1)
            else:
                gl = jnp.sum(xf * gw_ref[...], axis=-1, keepdims=True)
                gate = jax.nn.sigmoid(gl)
            out_v[pl.ds(r0, 2 * SEG), :] = (gate * a + bacc[pl.ds(r0, 2 * SEG), :]).astype(out_v.dtype)
            out_copy(i).start()
            return aB[:M]

        def multi_step(ii, mem):
            for uu in range(UNR):
                mem = pair_step(ii * UNR + uu, mem, uu > 0)
            return mem
        lax.fori_loop(0, NITRUN // UNR, multi_step, mem0_ref[...].astype(F32))
        def wait_out(i, c):
            out_copy(i).wait()
            return c
        lax.fori_loop(0, NITRUN, wait_out, 0)

    any_spec = pl.BlockSpec(memory_space=pl.ANY)
    out = pl.pallas_call(
        kernel,
        out_shape=jax.ShapeDtypeStruct((S, Dm), BF16),
        in_specs=[any_spec] * 10,
        out_specs=any_spec,
        scratch_shapes=[
            pltpu.VMEM((S // 2, Dm), U32), pltpu.VMEM((M, Dm), BF16), pltpu.VMEM((NG, 2 * JG, D2, Dh), U32),
            pltpu.VMEM((Df, Dm), U32),
            pltpu.VMEM((Df // 2, Dm), U32), pltpu.VMEM((Dm,), BF16), pltpu.VMEM((1, Dm), F32), pltpu.VMEM((S, Dm), BF16),
            pltpu.VMEM((D2, 3 * H * Dh), U32), pltpu.VMEM((H * Dh // 2, Dm), U32),
            pltpu.VMEM((S, Dm), F32), pltpu.VMEM((S, 128), F32), pltpu.VMEM((8, 3 * H * Dh), F32), pltpu.VMEM((8, H * Dh), F32),
            pltpu.SemaphoreType.DMA((NSEM,)), pltpu.SemaphoreType.DMA,
        ],
        compiler_params=pltpu.CompilerParams(vmem_limit_bytes=110 * 1024 * 1024, disable_bounds_checks=NOBC),
    )(A_x.reshape(S, Dm), A_mem0.reshape(M, Dm), A_Wq.reshape(D2, 2 * H, Dh), A_Wk.reshape(D2, 2 * H, Dh),
      A_Wv.reshape(D2, 2 * H, Dh), A_Wo.reshape(H * Dh, Dm),
      B_w_gate.T, B_w_up.T, B_w_down, gate_w)
    return out.reshape(B, S, Dm)


@jax.jit
def pallas_gated_mix__memory_aug_recurrent_mem_tr__glu_gated_geglu__prompt_kernel(
    A_x: jax.Array,
    A_mem0: jax.Array,
    A_Wq: jax.Array,
    A_Wk: jax.Array,
    A_Wv: jax.Array,
    A_Wo: jax.Array,
    A_seg_len: jax.Array,
    B_x: jax.Array,
    B_w_gate: jax.Array,
    B_w_up: jax.Array,
    B_w_down: jax.Array,
    gate_w: jax.Array,
):
    return _impl(A_x, A_mem0, A_Wq, A_Wk, A_Wv, A_Wo, A_seg_len, B_x, B_w_gate, B_w_up, B_w_down, gate_w)
```

```python
import functools

import jax
import jax.numpy as jnp
from jax import lax
import jax.experimental.pallas as pl
import jax.experimental.pallas.tpu as pltpu

F32 = jnp.float32
BF16 = jnp.bfloat16
U32 = jnp.uint32

_NT = (((1,), (1,)), ((), ()))


def _gelu_tanh(x):
    c = 0.7978845608028654
    return 0.5 * x * (1.0 + jnp.tanh(c * (x + 0.044715 * (x * x * x))))


def _recip(d):
    r = pl.reciprocal(d, approx=True)
    return r * (2.0 - d * r)


def _bf(w32):
    return pltpu.bitcast(w32, BF16)


def _dot(a, b):
    return jnp.dot(a, b, preferred_element_type=F32)


def _dot_nt(a, b):
    return lax.dot_general(a, b, _NT, preferred_element_type=F32)


def _impl(A_x, A_mem0, A_Wq, A_Wk, A_Wv, A_Wo, A_seg_len, B_x, B_w_gate, B_w_up, B_w_down, gate_w):
    del A_seg_len, B_x
    B, S, Dm = A_x.shape
    H, Dh = A_Wq.shape[1], A_Wq.shape[2]
    M = A_mem0.shape[1]
    Df = B_w_gate.shape[1]
    SEG = 32
    assert (B, S, Dm, H, Dh, M, Df) == (1, 2048, 640, 32, 128, 8, 1728)
    L = M + SEG
    NIT = S // (2 * SEG)
    UNR = 2
    scale = Dh ** (-0.5)
    NP = H // 2
    PW = 6 * Dh
    D2 = Dm // 2
    DS, DPV = 1, 2
    TAIL_A, TAIL_B = (2, 3, 4), (2, 2, 2)
    NTW = 3
    GB0, GB, FC = 512, 256, 256
    NG = (S - GB0) // GB
    JG = 3 * NP // NG
    GPW = NP // JG
    QSPLIT = 4
    fchunks = [(f0, min(FC, Df - f0)) for f0 in range(0, Df, FC)]
    NFC = len(fchunks)
    WAIT_PTS = (0, 1, 2, 5, 9)
    START_PTS = (1, 5)
    SEM_G = 5
    SEM_F = SEM_G + NG
    NSEM = SEM_F + 3 * NFC + 1

    def kernel(x_hbm, mem0_hbm, wq_hbm, wk_hbm, wv_hbm, wo_hbm, wgT_hbm, wuT_hbm, wd_hbm, gw_hbm,
               out_hbm,
               x32, mem0_ref, wst, wgu32, wd32, gw1_ref, gw_ref, out_v,
               wqkv32, wo32, bacc, gsv, qkv_sv, o_sv, sems, osem):
        def cp(src, dst, i):
            return pltpu.make_async_copy(src, dst, sems.at[i])

        x32h = x_hbm.bitcast(U32)
        c_x0 = cp(x32h.at[pl.ds(0, GB0 // 4)], x32.at[pl.ds(0, GB0 // 4)], 0)
        c_x1 = cp(x32h.at[pl.ds(GB0 // 4, GB0 // 4)], x32.at[pl.ds(GB0 // 4, GB0 // 4)], NSEM - 1)
        c_xr = cp(x32h.at[pl.ds(GB0 // 2, (S - GB0) // 2)], x32.at[pl.ds(GB0 // 2, (S - GB0) // 2)], 1)
        c_gw = cp(gw_hbm, gw1_ref, 2)
        c_m0 = cp(mem0_hbm, mem0_ref, 3)
        c_wo = cp(wo_hbm.bitcast(U32), wo32, 4)
        c_w = []
        for t, w_hbm in enumerate((wq_hbm, wk_hbm, wv_hbm)):
            w32 = w_hbm.bitcast(U32)
            for hf in range(GPW):
                gi = t * GPW + hf
                c_w.append([cp(w32.at[:, par * NP + hf * JG + jj, :], wst.at[gi, par * JG + jj], SEM_G + gi)
                            for jj in range(JG) for par in range(2)])
        wg32h, wu32h, wd32h = wgT_hbm.bitcast(U32), wuT_hbm.bitcast(U32), wd_hbm.bitcast(U32)
        c_f = [[], [], []]
        for c, (f0, fw) in enumerate(fchunks):
            src = pl.ds(f0 // 2, fw // 2)
            c_f[0].append(cp(wg32h.at[src], wgu32.at[pl.ds(f0, fw // 2)], SEM_F + c))
            c_f[1].append(cp(wu32h.at[src], wgu32.at[pl.ds(f0 + fw // 2, fw // 2)], SEM_F + NFC + c))
            c_f[2].append(cp(wd32h.at[src], wd32.at[src], SEM_F + 2 * NFC + c))

        def xrows(r0, n):
            if isinstance(r0, int):
                return _bf(x32[r0 // 2:(r0 + n) // 2, :])
            return _bf(x32[pl.ds(pl.multiple_of(r0 // 2, 8), n // 2), :])

        def relay(gi, jj):
            t = gi // GPW
            hf = gi % GPW
            off = pl.multiple_of((hf * JG + jj) * PW + t * 2 * Dh, 2 * Dh)
            for i0 in range(0, D2, 64):
                a = wst[gi, jj, i0:i0 + 64, :]
                b = wst[gi, JG + jj, i0:i0 + 64, :]
                lo = (a & U32(0xFFFF)) | (b << 16)
                hi = (a >> 16) | (b & U32(0xFFFF0000))
                wqkv32[i0:i0 + 64, pl.ds(off, Dh)] = lo
                wqkv32[i0:i0 + 64, pl.ds(off + Dh, Dh)] = hi

        def geglu(r0, nrows, before, jobs, ramp=False):
            nslots = 2 * NFC
            slot = [0]

            def filler():
                lo = slot[0] * len(jobs) // nslots
                hi = (slot[0] + 1) * len(jobs) // nslots
                for j in jobs[lo:hi]:
                    j()
                slot[0] += 1

            hs = {}
            b = None
            for c in range(NFC + 1):
                if c < NFC:
                    f0, fw = fchunks[c]
                    before(('gu', c))
                    if ramp and c == 0:
                        hr = nrows // 2
                        gu0 = _dot_nt(xrows(r0, hr), _bf(wgu32[f0:f0 + fw, :]))
                        c_x1.wait()
                        gu1 = _dot_nt(xrows(r0 + hr, hr), _bf(wgu32[f0:f0 + fw, :]))
                        gu = jnp.concatenate([gu0, gu1], axis=0)
                    else:
                        gu = _dot_nt(xrows(r0, nrows), _bf(wgu32[f0:f0 + fw, :]))
                    filler()
                    hs[c] = (_gelu_tanh(gu[:, :fw]) * gu[:, fw:]).astype(BF16)
                if c >= 1:
                    f0, fw = fchunks[c - 1]
                    hh = hs.pop(c - 1)
                    before(('d', c - 1))
                    if c == NFC and fw % 128 != 0:
                        k0 = fw // 128 * 128
                        b = b + _dot(hh[:, :k0], _bf(wd32[f0 // 2:(f0 + k0) // 2, :]))
                        wl = _bf(wd32[(f0 + k0) // 2:(f0 + fw) // 2, :])
                        qr = nrows // QSPLIT
                        r = jnp.concatenate([_dot(hh[q * qr:(q + 1) * qr, k0:], wl) for q in range(QSPLIT)], axis=0)
                    else:
                        r = _dot(hh, _bf(wd32[f0 // 2:(f0 + fw) // 2, :]))
                    b = r if b is None else b + r
                    filler()
            gate = jax.nn.sigmoid(jnp.sum(xrows(r0, nrows).astype(F32) * gw_ref[...], axis=-1, keepdims=True))
            bacc[pl.ds(r0, nrows), :] = (1.0 - gate) * b
            gsv[pl.ds(r0, nrows), :] = jnp.broadcast_to(gate, (nrows, 128))

        c_x0.start()
        c_f[0][0].start()
        c_f[1][0].start()
        c_x1.start()
        c_gw.start()
        c_m0.start()
        for c in range(1, NFC):
            c_f[0][c].start()
            c_f[1][c].start()
            c_f[2][c - 1].start()
        c_f[2][NFC - 1].start()
        c_xr.start()
        c_x0.wait()
        seq = [('gu', 0)]
        for c in range(1, NFC):
            seq += [('gu', c), ('d', c - 1)]
        seq.append(('d', NFC - 1))

        def before0(item):
            n = seq.index(item)
            if n in WAIT_PTS:
                nxt = [w for w in WAIT_PTS if w > n]
                end = nxt[0] if nxt else len(seq)
                for kind, cc in seq[n:end]:
                    if kind == 'gu':
                        c_f[0][cc].wait()
                        c_f[1][cc].wait()
                    else:
                        c_f[2][cc].wait()
            if n == WAIT_PTS[1]:
                c_gw.wait()
                c_m0.wait()
                gw_ref[...] = gw1_ref[...].astype(F32).reshape(1, Dm)
            if n in START_PTS:
                k = START_PTS.index(n)
                for gi in range(k * 2, k * 2 + 2):
                    for cc in c_w[gi]:
                        cc.start()

        geglu(0, GB0, before0, [], ramp=True)
        c_xr.wait()
        for gi in range(2 * len(START_PTS), NG):
            for cc in c_w[gi]:
                cc.start()
        c_wo.start()

        def geglu_loop(gi, carry):
            r0 = pl.multiple_of(GB0 + gi * GB, GB)
            pltpu.make_async_copy(wst.at[gi], wst.at[gi], sems.at[SEM_G + gi]).wait()
            jobs = [functools.partial(relay, gi, jj) for jj in range(JG)]
            geglu(r0, GB, lambda item: None, jobs)
            return carry

        lax.fori_loop(0, NG, geglu_loop, 0)
        c_wo.wait()

        ri = lax.broadcasted_iota(jnp.int32, (2 * L, 2 * L), 0)
        ci = lax.broadcasted_iota(jnp.int32, (2 * L, 2 * L), 1)
        rh = ri >= L
        ch = ci >= L
        rl = jnp.where(rh, ri - L, ri)
        cl = jnp.where(ch, ci - L, ci)
        mask = (rh == ch) & ((rl < M) | (rl >= cl))
        fill = jnp.where(rh == ch, -1e9, -jnp.inf).astype(F32)

        def seg_step(h, first, ksplit):
            qkv_s, e_s, o2_s = {}, {}, {}
            acc = [None]

            def do_qkv(p):
                if ksplit and p == 0:
                    r = None
                    for kk in range(Dm // 128):
                        rr = _dot(h[:, kk * 128:(kk + 1) * 128],
                                  _bf(wqkv32[kk * 64:(kk + 1) * 64, p * PW:(p + 1) * PW]))
                        r = rr if r is None else r + rr
                else:
                    r = _dot(h, _bf(wqkv32[:, p * PW:(p + 1) * PW]))
                if first:
                    qkv_sv[:, p * PW:(p + 1) * PW] = r[L:L + 8]
                    qkv = r[0:L]
                else:
                    qkv = jnp.concatenate([r[0:M], qkv_sv[:, p * PW:(p + 1) * PW], r[M:]], axis=0)
                q = jnp.concatenate([qkv[:, 0:Dh], qkv[:, Dh:2 * Dh]], axis=0).astype(BF16)
                k = jnp.concatenate([qkv[:, 2 * Dh:3 * Dh], qkv[:, 3 * Dh:4 * Dh]], axis=0).astype(BF16)
                v = jnp.concatenate([qkv[:, 4 * Dh:5 * Dh], qkv[:, 5 * Dh:6 * Dh]], axis=0).astype(BF16)
                qkv_s[p] = (q, k, v)

            def do_s(p):
                q, k, _ = qkv_s[p]
                sc = _dot_nt(q, k) * scale
                sc = jnp.where(mask, sc, fill)
                mx = jnp.max(sc, axis=-1, keepdims=True)
                e = jnp.exp(sc - mx)
                den = jnp.sum(e, axis=-1, keepdims=True)
                e_s[p] = (e.astype(BF16), _recip(den))

            def do_pv(p):
                e, r = e_s.pop(p)
                v = qkv_s.pop(p)[2]
                o = _dot(e, v) * r
                o2 = jnp.concatenate([o[0:L], o[L:2 * L]], axis=1)
                if first:
                    o_sv[:, p * 2 * Dh:(p + 1) * 2 * Dh] = o2[L - 8:L]
                    o2_s[p] = o2[0:L - 8].astype(BF16)
                else:
                    o2_s[p] = jnp.concatenate([o2, o_sv[:, p * 2 * Dh:(p + 1) * 2 * Dh]], axis=0).astype(BF16)

            def do_wo(p):
                r = _dot(o2_s.pop(p), _bf(wo32[p * Dh:(p + 1) * Dh, :]))
                acc[0] = r if acc[0] is None else acc[0] + r

            for p in range(NP):
                do_qkv(p)
                if p - DS >= 0:
                    do_s(p - DS)
                if p - DPV >= 0:
                    do_pv(p - DPV)
            tail = []
            for t in range(NP, NP + DPV):
                if t - DS < NP:
                    tail.append((do_s, t - DS))
                tail.append((do_pv, t - DPV))
            wo_next = 0
            for (fn, p), cnt in zip(tail, TAIL_A if first else TAIL_B):
                for _ in range(cnt):
                    do_wo(wo_next)
                    wo_next += 1
                fn(p)
            while wo_next < NP - NTW:
                do_wo(wo_next)
                wo_next += 1
            o2 = jnp.concatenate([o2_s.pop(p) for p in range(NP - NTW, NP)], axis=1)
            return acc[0] + _dot(o2, _bf(wo32[(NP - NTW) * Dh:NP * Dh, :]))

        def out_copy(i):
            r0 = pl.multiple_of(i * 2 * SEG, 2 * SEG)
            return pltpu.make_async_copy(out_v.at[pl.ds(r0, 2 * SEG)], out_hbm.at[pl.ds(r0, 2 * SEG)], osem)

        def pair_step(i, mem, ksplit_a):
            r0 = pl.multiple_of(i * 2 * SEG, 2 * SEG)
            xf = xrows(r0, 2 * SEG).astype(F32)
            hA = jnp.concatenate([mem, xf[0:SEG + 8]], axis=0).astype(BF16)
            aA = seg_step(hA, True, ksplit_a)
            hB = jnp.concatenate([aA[:M], xf[SEG + 8:]], axis=0).astype(BF16)
            aB = seg_step(hB, False, True)
            a = jnp.concatenate([aA[M:], aB[L:L + 8], aB[M:L]], axis=0)
            gate = jnp.concatenate([gsv[pl.ds(r0, 2 * SEG), :]] * (Dm // 128), axis=1)
            out_v[pl.ds(r0, 2 * SEG), :] = (gate * a + bacc[pl.ds(r0, 2 * SEG), :]).astype(out_v.dtype)
            out_copy(i).start()
            return aB[:M]

        def multi_step(ii, mem):
            for uu in range(UNR):
                mem = pair_step(ii * UNR + uu, mem, uu > 0)
            return mem

        lax.fori_loop(0, NIT // UNR, multi_step, mem0_ref[...].astype(F32))

        def wait_out(i, c):
            out_copy(i).wait()
            return c

        lax.fori_loop(0, NIT, wait_out, 0)

    any_spec = pl.BlockSpec(memory_space=pl.ANY)
    out = pl.pallas_call(
        kernel,
        out_shape=jax.ShapeDtypeStruct((S, Dm), BF16),
        in_specs=[any_spec] * 10,
        out_specs=any_spec,
        scratch_shapes=[
            pltpu.VMEM((S // 2, Dm), U32),
            pltpu.VMEM((M, Dm), BF16),
            pltpu.VMEM((NG, 2 * JG, D2, Dh), U32),
            pltpu.VMEM((Df, Dm), U32),
            pltpu.VMEM((Df // 2, Dm), U32),
            pltpu.VMEM((Dm,), BF16),
            pltpu.VMEM((1, Dm), F32),
            pltpu.VMEM((S, Dm), BF16),
            pltpu.VMEM((D2, 3 * H * Dh), U32),
            pltpu.VMEM((H * Dh // 2, Dm), U32),
            pltpu.VMEM((S, Dm), F32),
            pltpu.VMEM((S, 128), F32),
            pltpu.VMEM((8, 3 * H * Dh), F32),
            pltpu.VMEM((8, H * Dh), F32),
            pltpu.SemaphoreType.DMA((NSEM,)),
            pltpu.SemaphoreType.DMA,
        ],
        compiler_params=pltpu.CompilerParams(vmem_limit_bytes=110 * 1024 * 1024, disable_bounds_checks=True),
    )(A_x.reshape(S, Dm), A_mem0.reshape(M, Dm),
      A_Wq.reshape(D2, 2 * H, Dh), A_Wk.reshape(D2, 2 * H, Dh), A_Wv.reshape(D2, 2 * H, Dh),
      A_Wo.reshape(H * Dh, Dm), B_w_gate.T, B_w_up.T, B_w_down, gate_w)
    return out.reshape(B, S, Dm)


@jax.jit
def pallas_gated_mix__memory_aug_recurrent_mem_tr__glu_gated_geglu__prompt_kernel(
    A_x: jax.Array,
    A_mem0: jax.Array,
    A_Wq: jax.Array,
    A_Wk: jax.Array,
    A_Wv: jax.Array,
    A_Wo: jax.Array,
    A_seg_len: jax.Array,
    B_x: jax.Array,
    B_w_gate: jax.Array,
    B_w_up: jax.Array,
    B_w_down: jax.Array,
    gate_w: jax.Array,
):
    return _impl(A_x, A_mem0, A_Wq, A_Wk, A_Wv, A_Wo, A_seg_len, B_x, B_w_gate, B_w_up, B_w_down, gate_w)
```

```python
import functools

import jax
import jax.numpy as jnp
from jax import lax
import jax.experimental.pallas as pl
import jax.experimental.pallas.tpu as pltpu

F32 = jnp.float32
BF16 = jnp.bfloat16
U32 = jnp.uint32

_NT = (((1,), (1,)), ((), ()))


def _gelu_tanh(x):
    c = 0.7978845608028654
    return 0.5 * x * (1.0 + jnp.tanh(c * (x + 0.044715 * (x * x * x))))


def _recip(d):
    r = pl.reciprocal(d, approx=True)
    return r * (2.0 - d * r)


def _bf(w32):
    return pltpu.bitcast(w32, BF16)


def _compiler_params():
    kw = dict(vmem_limit_bytes=110 * 1024 * 1024)
    for extra in ("disable_bounds_checks", "disable_semaphore_checks"):
        try:
            pltpu.CompilerParams(**{extra: True})
            kw[extra] = True
        except TypeError:
            pass
    return pltpu.CompilerParams(**kw)


def _dot(a, b):
    return jnp.dot(a, b, preferred_element_type=F32)


def _dot_nt(a, b):
    return lax.dot_general(a, b, _NT, preferred_element_type=F32)


def _impl(A_x, A_mem0, A_Wq, A_Wk, A_Wv, A_Wo, A_seg_len, B_x, B_w_gate, B_w_up, B_w_down, gate_w):
    del A_seg_len, B_x
    B, S, Dm = A_x.shape
    H, Dh = A_Wq.shape[1], A_Wq.shape[2]
    M = A_mem0.shape[1]
    Df = B_w_gate.shape[1]
    SEG = 32
    assert (B, S, Dm, H, Dh, M, Df) == (1, 2048, 640, 32, 128, 8, 1728)
    L = M + SEG
    NIT = S // (2 * SEG)
    UNR = 2
    scale = Dh ** (-0.5)
    NP = H // 2
    PW = 6 * Dh
    D2 = Dm // 2
    DS, DPV = 1, 2
    TAIL_A, TAIL_B = (2, 3, 4), (2, 2, 2)
    NTW = 3
    GB0, GB, FC = 512, 256, 256
    NG = (S - GB0) // GB
    JG = 3 * NP // NG
    GPW = NP // JG
    QSPLIT = 4
    fchunks = [(f0, min(FC, Df - f0)) for f0 in range(0, Df, FC)]
    NFC = len(fchunks)
    WAIT_PTS = (0, 1, 2, 5, 9)
    START_PTS = (1, 5)
    SEM_G = 5
    SEM_F = SEM_G + NG
    NSEM = SEM_F + 3 * NFC + 1

    def kernel(x_hbm, mem0_hbm, wq_hbm, wk_hbm, wv_hbm, wo_hbm, wgT_hbm, wuT_hbm, wd_hbm, gw_hbm,
               out_hbm,
               x32, mem0_ref, wst, wgu32, wd32, gw1_ref, gw_ref, out_v,
               wqkv32, wo32, bacc, gsv, qkv_sv, o_sv, sems, osem):
        def cp(src, dst, i):
            return pltpu.make_async_copy(src, dst, sems.at[i])

        x32h = x_hbm.bitcast(U32)
        c_x0 = cp(x32h.at[pl.ds(0, GB0 // 4)], x32.at[pl.ds(0, GB0 // 4)], 0)
        c_x1 = cp(x32h.at[pl.ds(GB0 // 4, GB0 // 4)], x32.at[pl.ds(GB0 // 4, GB0 // 4)], NSEM - 1)
        c_xr = cp(x32h.at[pl.ds(GB0 // 2, (S - GB0) // 2)], x32.at[pl.ds(GB0 // 2, (S - GB0) // 2)], 1)
        c_gw = cp(gw_hbm, gw1_ref, 2)
        c_m0 = cp(mem0_hbm, mem0_ref, 3)
        c_wo = cp(wo_hbm.bitcast(U32), wo32, 4)
        c_w = []
        for t, w_hbm in enumerate((wq_hbm, wk_hbm, wv_hbm)):
            w32 = w_hbm.bitcast(U32)
            for hf in range(GPW):
                gi = t * GPW + hf
                c_w.append([cp(w32.at[:, par * NP + hf * JG + jj, :], wst.at[gi, par * JG + jj], SEM_G + gi)
                            for jj in range(JG) for par in range(2)])
        wg32h, wu32h, wd32h = wgT_hbm.bitcast(U32), wuT_hbm.bitcast(U32), wd_hbm.bitcast(U32)
        c_f = [[], [], []]
        for c, (f0, fw) in enumerate(fchunks):
            src = pl.ds(f0 // 2, fw // 2)
            c_f[0].append(cp(wg32h.at[src], wgu32.at[pl.ds(f0, fw // 2)], SEM_F + c))
            c_f[1].append(cp(wu32h.at[src], wgu32.at[pl.ds(f0 + fw // 2, fw // 2)], SEM_F + NFC + c))
            c_f[2].append(cp(wd32h.at[src], wd32.at[src], SEM_F + 2 * NFC + c))

        def xrows(r0, n):
            if isinstance(r0, int):
                return _bf(x32[r0 // 2:(r0 + n) // 2, :])
            return _bf(x32[pl.ds(pl.multiple_of(r0 // 2, 8), n // 2), :])

        def relay(gi, jj):
            t = gi // GPW
            hf = gi % GPW
            off = pl.multiple_of((hf * JG + jj) * PW + t * 2 * Dh, 2 * Dh)
            for i0 in range(0, D2, 64):
                a = wst[gi, jj, i0:i0 + 64, :]
                b = wst[gi, JG + jj, i0:i0 + 64, :]
                lo = (a & U32(0xFFFF)) | (b << 16)
                hi = (a >> 16) | (b & U32(0xFFFF0000))
                wqkv32[i0:i0 + 64, pl.ds(off, Dh)] = lo
                wqkv32[i0:i0 + 64, pl.ds(off + Dh, Dh)] = hi

        def geglu(r0, nrows, before, jobs, ramp=False):
            nslots = 2 * NFC
            slot = [0]

            def filler():
                lo = slot[0] * len(jobs) // nslots
                hi = (slot[0] + 1) * len(jobs) // nslots
                for j in jobs[lo:hi]:
                    j()
                slot[0] += 1

            hs = {}
            b = None
            for c in range(NFC + 1):
                if c < NFC:
                    f0, fw = fchunks[c]
                    before(('gu', c))
                    if ramp and c == 0:
                        hr = nrows // 2
                        gu0 = _dot_nt(xrows(r0, hr), _bf(wgu32[f0:f0 + fw, :]))
                        c_x1.wait()
                        gu1 = _dot_nt(xrows(r0 + hr, hr), _bf(wgu32[f0:f0 + fw, :]))
                        gu = jnp.concatenate([gu0, gu1], axis=0)
                    else:
                        gu = _dot_nt(xrows(r0, nrows), _bf(wgu32[f0:f0 + fw, :]))
                    filler()
                    hs[c] = (_gelu_tanh(gu[:, :fw]) * gu[:, fw:]).astype(BF16)
                if c >= 1:
                    f0, fw = fchunks[c - 1]
                    hh = hs.pop(c - 1)
                    before(('d', c - 1))
                    if c == NFC and fw % 128 != 0:
                        k0 = fw // 128 * 128
                        b = b + _dot(hh[:, :k0], _bf(wd32[f0 // 2:(f0 + k0) // 2, :]))
                        wl = _bf(wd32[(f0 + k0) // 2:(f0 + fw) // 2, :])
                        qr = nrows // QSPLIT
                        r = jnp.concatenate([_dot(hh[q * qr:(q + 1) * qr, k0:], wl) for q in range(QSPLIT)], axis=0)
                    else:
                        r = _dot(hh, _bf(wd32[f0 // 2:(f0 + fw) // 2, :]))
                    b = r if b is None else b + r
                    filler()
            gate = jax.nn.sigmoid(jnp.sum(xrows(r0, nrows).astype(F32) * gw_ref[...], axis=-1, keepdims=True))
            bacc[pl.ds(r0, nrows), :] = (1.0 - gate) * b
            gsv[pl.ds(r0, nrows), :] = jnp.broadcast_to(gate, (nrows, 128))

        c_x0.start()
        c_f[0][0].start()
        c_f[1][0].start()
        c_x1.start()
        c_gw.start()
        c_m0.start()
        for c in range(1, NFC):
            c_f[0][c].start()
            c_f[1][c].start()
            c_f[2][c - 1].start()
        c_f[2][NFC - 1].start()
        c_xr.start()
        c_x0.wait()
        seq = [('gu', 0)]
        for c in range(1, NFC):
            seq += [('gu', c), ('d', c - 1)]
        seq.append(('d', NFC - 1))

        def before0(item):
            n = seq.index(item)
            if n in WAIT_PTS:
                nxt = [w for w in WAIT_PTS if w > n]
                end = nxt[0] if nxt else len(seq)
                for kind, cc in seq[n:end]:
                    if kind == 'gu':
                        c_f[0][cc].wait()
                        c_f[1][cc].wait()
                    else:
                        c_f[2][cc].wait()
            if n == WAIT_PTS[1]:
                c_gw.wait()
                c_m0.wait()
                gw_ref[...] = gw1_ref[...].astype(F32).reshape(1, Dm)
            if n in START_PTS:
                k = START_PTS.index(n)
                for gi in range(k * 2, k * 2 + 2):
                    for cc in c_w[gi]:
                        cc.start()

        geglu(0, GB0, before0, [], ramp=True)
        c_xr.wait()
        for gi in range(2 * len(START_PTS), NG):
            for cc in c_w[gi]:
                cc.start()
        c_wo.start()

        def geglu_loop(gi, carry):
            r0 = pl.multiple_of(GB0 + gi * GB, GB)
            pltpu.make_async_copy(wst.at[gi], wst.at[gi], sems.at[SEM_G + gi]).wait()
            jobs = [functools.partial(relay, gi, jj) for jj in range(JG)]
            geglu(r0, GB, lambda item: None, jobs)
            return carry

        lax.fori_loop(0, NG, geglu_loop, 0)
        c_wo.wait()

        ri = lax.broadcasted_iota(jnp.int32, (2 * L, 2 * L), 0)
        ci = lax.broadcasted_iota(jnp.int32, (2 * L, 2 * L), 1)
        rh = ri >= L
        ch = ci >= L
        rl = jnp.where(rh, ri - L, ri)
        cl = jnp.where(ch, ci - L, ci)
        mask = (rh == ch) & ((rl < M) | (rl >= cl))
        fill = jnp.where(rh == ch, -1e9, -jnp.inf).astype(F32)

        def seg_step(h, first, ksplit):
            qkv_s, e_s, o2_s = {}, {}, {}
            acc = [None]

            def do_qkv(p):
                if ksplit and p == 0:
                    r = None
                    for kk in range(Dm // 128):
                        rr = _dot(h[:, kk * 128:(kk + 1) * 128],
                                  _bf(wqkv32[kk * 64:(kk + 1) * 64, p * PW:(p + 1) * PW]))
                        r = rr if r is None else r + rr
                else:
                    r = _dot(h, _bf(wqkv32[:, p * PW:(p + 1) * PW]))
                if first:
                    qkv_sv[:, p * PW:(p + 1) * PW] = r[L:L + 8]
                    qkv = r[0:L]
                else:
                    qkv = jnp.concatenate([r[0:M], qkv_sv[:, p * PW:(p + 1) * PW], r[M:]], axis=0)
                q = jnp.concatenate([qkv[:, 0:Dh], qkv[:, Dh:2 * Dh]], axis=0).astype(BF16)
                k = jnp.concatenate([qkv[:, 2 * Dh:3 * Dh], qkv[:, 3 * Dh:4 * Dh]], axis=0).astype(BF16)
                v = jnp.concatenate([qkv[:, 4 * Dh:5 * Dh], qkv[:, 5 * Dh:6 * Dh]], axis=0).astype(BF16)
                qkv_s[p] = (q, k, v)

            def do_s(p):
                q, k, _ = qkv_s[p]
                sc = _dot_nt(q, k) * scale
                sc = jnp.where(mask, sc, fill)
                mx = jnp.max(sc, axis=-1, keepdims=True)
                e = jnp.exp(sc - mx)
                den = jnp.sum(e, axis=-1, keepdims=True)
                e_s[p] = (e.astype(BF16), _recip(den))

            def do_pv(p):
                e, r = e_s.pop(p)
                v = qkv_s.pop(p)[2]
                o = _dot(e, v) * r
                o2 = jnp.concatenate([o[0:L], o[L:2 * L]], axis=1)
                if first:
                    o_sv[:, p * 2 * Dh:(p + 1) * 2 * Dh] = o2[L - 8:L]
                    o2_s[p] = o2[0:L - 8].astype(BF16)
                else:
                    o2_s[p] = jnp.concatenate([o2, o_sv[:, p * 2 * Dh:(p + 1) * 2 * Dh]], axis=0).astype(BF16)

            def do_wo(p):
                r = _dot(o2_s.pop(p), _bf(wo32[p * Dh:(p + 1) * Dh, :]))
                acc[0] = r if acc[0] is None else acc[0] + r

            for p in range(NP):
                do_qkv(p)
                if p - DS >= 0:
                    do_s(p - DS)
                if p - DPV >= 0:
                    do_pv(p - DPV)
            tail = []
            for t in range(NP, NP + DPV):
                if t - DS < NP:
                    tail.append((do_s, t - DS))
                tail.append((do_pv, t - DPV))
            wo_next = 0
            for (fn, p), cnt in zip(tail, TAIL_A if first else TAIL_B):
                for _ in range(cnt):
                    do_wo(wo_next)
                    wo_next += 1
                fn(p)
            while wo_next < NP - NTW:
                do_wo(wo_next)
                wo_next += 1
            o2 = jnp.concatenate([o2_s.pop(p) for p in range(NP - NTW, NP)], axis=1)
            return acc[0] + _dot(o2, _bf(wo32[(NP - NTW) * Dh:NP * Dh, :]))

        def out_copy(i):
            r0 = pl.multiple_of(i * 2 * SEG, 2 * SEG)
            return pltpu.make_async_copy(out_v.at[pl.ds(r0, 2 * SEG)], out_hbm.at[pl.ds(r0, 2 * SEG)], osem)

        def pair_step(i, mem, ksplit_a):
            r0 = pl.multiple_of(i * 2 * SEG, 2 * SEG)
            xf = xrows(r0, 2 * SEG).astype(F32)
            hA = jnp.concatenate([mem, xf[0:SEG + 8]], axis=0).astype(BF16)
            aA = seg_step(hA, True, ksplit_a)
            hB = jnp.concatenate([aA[:M], xf[SEG + 8:]], axis=0).astype(BF16)
            aB = seg_step(hB, False, True)
            a = jnp.concatenate([aA[M:], aB[L:L + 8], aB[M:L]], axis=0)
            gate = jnp.concatenate([gsv[pl.ds(r0, 2 * SEG), :]] * (Dm // 128), axis=1)
            out_v[pl.ds(r0, 2 * SEG), :] = (gate * a + bacc[pl.ds(r0, 2 * SEG), :]).astype(out_v.dtype)
            out_copy(i).start()
            return aB[:M]

        def multi_step(ii, mem):
            for uu in range(UNR):
                mem = pair_step(ii * UNR + uu, mem, uu > 0)
            return mem

        lax.fori_loop(0, NIT // UNR, multi_step, mem0_ref[...].astype(F32))

        def wait_out(i, c):
            out_copy(i).wait()
            return c

        lax.fori_loop(0, NIT, wait_out, 0)

    any_spec = pl.BlockSpec(memory_space=pl.ANY)
    out = pl.pallas_call(
        kernel,
        out_shape=jax.ShapeDtypeStruct((S, Dm), BF16),
        in_specs=[any_spec] * 10,
        out_specs=any_spec,
        scratch_shapes=[
            pltpu.VMEM((S // 2, Dm), U32),
            pltpu.VMEM((M, Dm), BF16),
            pltpu.VMEM((NG, 2 * JG, D2, Dh), U32),
            pltpu.VMEM((Df, Dm), U32),
            pltpu.VMEM((Df // 2, Dm), U32),
            pltpu.VMEM((Dm,), BF16),
            pltpu.VMEM((1, Dm), F32),
            pltpu.VMEM((S, Dm), BF16),
            pltpu.VMEM((D2, 3 * H * Dh), U32),
            pltpu.VMEM((H * Dh // 2, Dm), U32),
            pltpu.VMEM((S, Dm), F32),
            pltpu.VMEM((S, 128), F32),
            pltpu.VMEM((8, 3 * H * Dh), F32),
            pltpu.VMEM((8, H * Dh), F32),
            pltpu.SemaphoreType.DMA((NSEM,)),
            pltpu.SemaphoreType.DMA,
        ],
        compiler_params=_compiler_params(),
    )(A_x.reshape(S, Dm), A_mem0.reshape(M, Dm),
      A_Wq.reshape(D2, 2 * H, Dh), A_Wk.reshape(D2, 2 * H, Dh), A_Wv.reshape(D2, 2 * H, Dh),
      A_Wo.reshape(H * Dh, Dm), B_w_gate.T, B_w_up.T, B_w_down, gate_w)
    return out.reshape(B, S, Dm)


@jax.jit
def pallas_gated_mix__memory_aug_recurrent_mem_tr__glu_gated_geglu__prompt_kernel(
    A_x: jax.Array,
    A_mem0: jax.Array,
    A_Wq: jax.Array,
    A_Wk: jax.Array,
    A_Wv: jax.Array,
    A_Wo: jax.Array,
    A_seg_len: jax.Array,
    B_x: jax.Array,
    B_w_gate: jax.Array,
    B_w_up: jax.Array,
    B_w_down: jax.Array,
    gate_w: jax.Array,
):
    return _impl(A_x, A_mem0, A_Wq, A_Wk, A_Wv, A_Wo, A_seg_len, B_x, B_w_gate, B_w_up, B_w_down, gate_w)
```
